```python
import jax
import jax.numpy as jnp

def _softmax(x, axis=-1):
    return jax.nn.softmax(x, axis=axis)
def _gelu(x):
    return jax.nn.gelu(x, approximate=True)
def _silu(x):
    return jax.nn.silu(x)
def _sigmoid(x):
    return jax.nn.sigmoid(x)
def _layernorm(x, axis=-1, eps=1e-5):
    m = jnp.mean(x, axis=axis, keepdims=True)
    v = jnp.var(x, axis=axis, keepdims=True)
    return (x - m) / jnp.sqrt(v + eps)
def _scatter_add(tgt, idx, src, axis=0):
    return tgt.at[idx].add(src)
def _segment_sum(src, seg, n):
    return jax.ops.segment_sum(src, seg, n)
class _Rng:
    def __init__(self, key):
        self._k = key
    def _next(self):
        self._k, sub = jax.random.split(self._k)
        return sub
    def normal(self, shape):
        return jax.random.normal(self._next(), shape, dtype=jnp.bfloat16)
    def randint(self, lo, hi, shape):
        return jax.random.randint(self._next(), shape, lo, hi, dtype=jnp.int32)
    def uniform(self, shape, lo=0.0, hi=1.0):
        return jax.random.uniform(self._next(), shape, jnp.bfloat16, lo, hi)
    def permutation(self, n):
        return jax.random.permutation(self._next(), n)


kernel_name = 'concat_heads__gqa_block_cached__gqa_block_cached__near_ridge'

def setup_inputs():
    _rng = _Rng(jax.random.key(int.from_bytes(__import__("os").urandom(4), "little")))
    _w = (lambda a: (lambda t: t.astype(jnp.bfloat16) if jnp.issubdtype(t.dtype, jnp.floating) else t)(jnp.asarray(a)))
    def _A_setup():
        B, Sq, D = 8, 256, 640
        Hq, Hkv, Sk, Dh = 32, 32, 1024, 192
        assert Hq % Hkv == 0, (Hq, Hkv)
        return {
            "x": _w((lambda *s: _rng.normal(s) * 0.05)(B, Sq, D)),
            "k_cache": _w((lambda *s: _rng.normal(s) * 0.05)(B, Hkv, Sk, Dh)),
            "v_cache": _w((lambda *s: _rng.normal(s) * 0.05)(B, Hkv, Sk, Dh)),
            "wq": _w((lambda *s: _rng.normal(s) * 0.05)(D, Hq * Dh) * (D ** -0.5)),
            "wo": _w((lambda *s: _rng.normal(s) * 0.05)(Hq * Dh, D) * ((Hq * Dh) ** -0.5)),
        }
    _A_in = _A_setup()

    def _B_setup():
        B, Sq, D = 8, 256, 640
        Hq, Hkv, Sk, Dh = 32, 32, 1024, 192
        assert Hq % Hkv == 0, (Hq, Hkv)
        return {
            "x": _w((lambda *s: _rng.normal(s) * 0.05)(B, Sq, D)),
            "k_cache": _w((lambda *s: _rng.normal(s) * 0.05)(B, Hkv, Sk, Dh)),
            "v_cache": _w((lambda *s: _rng.normal(s) * 0.05)(B, Hkv, Sk, Dh)),
            "wq": _w((lambda *s: _rng.normal(s) * 0.05)(D, Hq * Dh) * (D ** -0.5)),
            "wo": _w((lambda *s: _rng.normal(s) * 0.05)(Hq * Dh, D) * ((Hq * Dh) ** -0.5)),
        }
    _B_in = _B_setup()

    return {
        "A_x": _A_in["x"],
        "A_k_cache": _A_in["k_cache"],
        "A_v_cache": _A_in["v_cache"],
        "A_wq": _A_in["wq"],
        "A_wo": _A_in["wo"],
        "B_x": _B_in["x"],
        "B_k_cache": _B_in["k_cache"],
        "B_v_cache": _B_in["v_cache"],
        "B_wq": _B_in["wq"],
        "B_wo": _B_in["wo"],
    }

def reference(A_x, A_k_cache, A_v_cache, A_wq, A_wo, B_x, B_k_cache, B_v_cache, B_wq, B_wo):
    def _A_ref(x, k_cache, v_cache, wq, wo):
        B, Sq, D = x.shape
        Hq, Dh = 32, 192
        Hkv = k_cache.shape[1]
        rep = Hq // Hkv
        q = (lambda x, *d: x.transpose(*d))((x @ wq).reshape(B, Sq, Hq, Dh), 0, 2, 1, 3)
        k = jnp.repeat(k_cache, rep, axis=1)
        v = jnp.repeat(v_cache, rep, axis=1)
        scores = jnp.einsum("bhqd,bhkd->bhqk", q, k) * (Dh ** -0.5)
        p = _softmax(scores, axis=-1)
        o = jnp.einsum("bhqk,bhkd->bhqd", p, v)
        return (lambda x, *d: x.transpose(*d))(o, 0, 2, 1, 3).reshape(B, Sq, Hq * Dh) @ wo

    def _B_ref(x, k_cache, v_cache, wq, wo):
        B, Sq, D = x.shape
        Hq, Dh = 32, 192
        Hkv = k_cache.shape[1]
        rep = Hq // Hkv
        q = (lambda x, *d: x.transpose(*d))((x @ wq).reshape(B, Sq, Hq, Dh), 0, 2, 1, 3)
        k = jnp.repeat(k_cache, rep, axis=1)
        v = jnp.repeat(v_cache, rep, axis=1)
        scores = jnp.einsum("bhqd,bhkd->bhqk", q, k) * (Dh ** -0.5)
        p = _softmax(scores, axis=-1)
        o = jnp.einsum("bhqk,bhkd->bhqd", p, v)
        return (lambda x, *d: x.transpose(*d))(o, 0, 2, 1, 3).reshape(B, Sq, Hq * Dh) @ wo

    a = _A_ref(A_x, A_k_cache, A_v_cache, A_wq, A_wo)
    b = _B_ref(B_x, B_k_cache, B_v_cache, B_wq, B_wo)
    return jnp.concatenate([a, b], axis=-1)
```

```python
import functools
import math

import jax
import jax.numpy as jnp
import jax.experimental.pallas as pl
import jax.experimental.pallas.tpu as pltpu

HQ = 32
DH = 192
HB = 2

_NT = (((1,), (1,)), ((), ()))
_TN = (((0,), (0,)), ((), ()))


def _branch(x_ref, kt_ref, vt_ref, wq_ref, wo_ref, acc_ref, b, col0, hb):
    c = (DH ** -0.5) * math.log2(math.e)
    x = x_ref[b]
    q = jnp.dot(x, wq_ref[...], preferred_element_type=jnp.float32)
    q = (q * c).astype(jnp.bfloat16)
    outs = []
    for h in range(hb):
        qh = q[:, h * DH:(h + 1) * DH]
        s = jnp.dot(qh, kt_ref[0, h], preferred_element_type=jnp.float32)
        m = jnp.max(s, axis=-1, keepdims=True)
        p = jnp.exp2(s - m)
        l = jnp.sum(p, axis=-1, keepdims=True)
        ot = jax.lax.dot_general(vt_ref[0, h], p.astype(jnp.bfloat16), _NT,
                                 preferred_element_type=jnp.float32)
        lt = jnp.transpose(jnp.broadcast_to(l, (l.shape[0], 128)))[0:1, :]
        outs.append((ot * (1.0 / lt)).astype(jnp.bfloat16))
    ot = jnp.concatenate(outs, axis=0)
    y = jax.lax.dot_general(ot, wo_ref[...], _TN, preferred_element_type=jnp.float32)
    d = y.shape[1]
    acc_ref[b, :, col0:col0 + d] += y


def _kernel(xa_ref, xb_ref, ka_ref, va_ref, kb_ref, vb_ref, wqa_ref, wqb_ref,
            woa_ref, wob_ref, out_ref, acc_ref, *, hb):
    g = pl.program_id(0)
    b = pl.program_id(1)

    @pl.when(g == 0)
    def _():
        acc_ref[b] = jnp.zeros(acc_ref.shape[1:], acc_ref.dtype)

    d = xa_ref.shape[2]
    _branch(xa_ref, ka_ref, va_ref, wqa_ref, woa_ref, acc_ref, b, 0, hb)
    _branch(xb_ref, kb_ref, vb_ref, wqb_ref, wob_ref, acc_ref, b, d, hb)

    @pl.when(g == pl.num_programs(0) - 1)
    def _():
        out_ref[b] = acc_ref[b].astype(out_ref.dtype)


@jax.jit
def pallas_concat_heads__gqa_block_cached__gqa_block_cached__near_ridge_kernel(
    A_x: jax.Array,
    A_k_cache: jax.Array,
    A_v_cache: jax.Array,
    A_wq: jax.Array,
    A_wo: jax.Array,
    B_x: jax.Array,
    B_k_cache: jax.Array,
    B_v_cache: jax.Array,
    B_wq: jax.Array,
    B_wo: jax.Array,
):
    B, Sq, D = A_x.shape
    _, H, Sk, Dh = A_k_cache.shape
    hb = HB
    kt_a = jnp.swapaxes(A_k_cache, -1, -2)
    vt_a = jnp.swapaxes(A_v_cache, -1, -2)
    kt_b = jnp.swapaxes(B_k_cache, -1, -2)
    vt_b = jnp.swapaxes(B_v_cache, -1, -2)

    x_spec = pl.BlockSpec((B, Sq, D), lambda g, b: (0, 0, 0))
    kv_spec = pl.BlockSpec((1, hb, Dh, Sk), lambda g, b: (b, g, 0, 0))
    wq_spec = pl.BlockSpec((D, hb * Dh), lambda g, b: (0, g))
    wo_spec = pl.BlockSpec((hb * Dh, D), lambda g, b: (g, 0))
    out_spec = pl.BlockSpec((B, Sq, 2 * D), lambda g, b: (0, 0, 0))

    return pl.pallas_call(
        functools.partial(_kernel, hb=hb),
        grid=(H // hb, B),
        in_specs=[x_spec, x_spec, kv_spec, kv_spec, kv_spec, kv_spec,
                  wq_spec, wq_spec, wo_spec, wo_spec],
        out_specs=out_spec,
        out_shape=jax.ShapeDtypeStruct((B, Sq, 2 * D), A_x.dtype),
        scratch_shapes=[pltpu.VMEM((B, Sq, 2 * D), jnp.float32)],
        compiler_params=pltpu.CompilerParams(
            dimension_semantics=("arbitrary", "arbitrary"),
            vmem_limit_bytes=100 * 1024 * 1024,
        ),
    )(A_x, B_x, kt_a, vt_a, kt_b, vt_b, A_wq, B_wq, A_wo, B_wo)
```

```python
import functools
import math
import os

import jax
import jax.numpy as jnp
import jax.experimental.pallas as pl
import jax.experimental.pallas.tpu as pltpu

DH = 192
AH = int('2')
HB = int(os.environ.get('HB', '4'))
NSLOT = int(os.environ.get('NSLOT', '2'))
HOOK = int('2')

_NT = (((1,), (1,)), ((), ()))
_TN = (((0,), (0,)), ((), ()))


def _kernel(xa_hbm, xb_hbm, ka_hbm, va_hbm, kb_hbm, vb_hbm,
            wqa_hbm, wqb_hbm, woa_hbm, wob_hbm, out_hbm,
            x_buf, k_buf, v_buf, wq_buf, wo_buf, acc_ref, o_buf,
            x_sem, kv_sem, w_sem, o_sem, fkv_sem, fw_sem, *, hb, nslot):
    nb, _, d = xa_hbm.shape
    ng = ka_hbm.shape[1] // hb
    nstep = ng * nb
    npair = hb // 2
    pw = 2 * DH
    c = (DH ** -0.5) * math.log2(math.e)
    x_hbm = (xa_hbm, xb_hbm)
    kv_hbm = ((ka_hbm, kb_hbm), (va_hbm, vb_hbm))
    kv_buf = (k_buf, v_buf)
    wq_hbm = (wqa_hbm, wqb_hbm)
    wo_hbm = (woa_hbm, wob_hbm)
    pairs = [(br, p) for p in range(npair) for br in range(2)]
    heads = [(br, 2 * p + j) for br, p in pairs for j in range(2)]
    n = len(heads)
    ahead = nslot - 1

    def x_copy(br, b):
        return pltpu.make_async_copy(x_hbm[br].at[b], x_buf.at[br, b], x_sem.at[br, b])

    def kv_copies(g, b, slot):
        hs = pl.ds(g * hb, hb)
        return [pltpu.make_async_copy(kv_hbm[j][br].at[b, hs], kv_buf[j].at[slot, br], kv_sem.at[slot, br, j])
                for br in range(2) for j in range(2)]

    def w_copies(g, slot):
        cs = pl.ds(pl.multiple_of(g * (hb * DH), 128), hb * DH)
        out = []
        for br in range(2):
            out.append(pltpu.make_async_copy(wq_hbm[br].at[:, cs], wq_buf.at[slot, br], w_sem.at[slot, br, 0]))
            out.append(pltpu.make_async_copy(wo_hbm[br].at[cs, :], wo_buf.at[slot, br], w_sem.at[slot, br, 1]))
        return out

    def o_copy(b):
        return pltpu.make_async_copy(o_buf.at[b], out_hbm.at[b], o_sem.at[b])

    def fkv_copy(j, br, p):
        hs = pl.ds(2 * p, 2)
        return pltpu.make_async_copy(kv_hbm[j][br].at[0, hs], kv_buf[j].at[0, br, hs], fkv_sem.at[j, br, p])

    def fq_copy(br, p):
        cs = pl.ds(p * pw, pw)
        return pltpu.make_async_copy(wq_hbm[br].at[:, cs], wq_buf.at[0, br, :, cs], fw_sem.at[0, br, p])

    def fo_copy(br, p):
        cs = pl.ds(p * pw, pw)
        return pltpu.make_async_copy(wo_hbm[br].at[cs, :], wo_buf.at[0, br, cs, :], fw_sem.at[1, br, p])

    def first_group(j):
        if j < 0:
            return [x_copy(0, 0), fq_copy(*pairs[0]), x_copy(1, 0), fq_copy(*pairs[1])]
        out = [fkv_copy(0, *pairs[j])]
        if j + 2 < len(pairs):
            out.append(fq_copy(*pairs[j + 2]))
        out += [fkv_copy(1, *pairs[j]), fo_copy(*pairs[j])]
        return out

    def body(b, slot, wslot, first, hook=None):
        def qproj(br, p):
            q = jnp.dot(x_buf[br, b], wq_buf[wslot, br, :, p * pw:(p + 1) * pw],
                        preferred_element_type=jnp.float32)
            return (q * c).astype(jnp.bfloat16)

        def scores(q, br, h):
            return jnp.dot(q[:, (h % 2) * DH:(h % 2 + 1) * DH], k_buf[slot, br, h],
                           preferred_element_type=jnp.float32)

        def softmax(s):
            m = jnp.max(s, axis=-1, keepdims=True)
            p = jnp.exp2(s - m)
            l = jnp.sum(p, axis=-1, keepdims=True)
            lt = jnp.transpose(jnp.broadcast_to(l, (l.shape[0], 128)))[0:1, :]
            return p.astype(jnp.bfloat16), 1.0 / lt

        def pv(pr, br, h):
            p, r = pr
            ot = jax.lax.dot_general(v_buf[slot, br, h], p, _NT, preferred_element_type=jnp.float32)
            return (ot * r).astype(jnp.bfloat16)

        def oproj(outs, br, p):
            ot = jnp.concatenate(outs, axis=0)
            y = jax.lax.dot_general(ot, wo_buf[wslot, br, p * pw:(p + 1) * pw, :], _TN,
                                    preferred_element_type=jnp.float32)
            acc_ref[b, :, br * d:(br + 1) * d] += y

        def wait_group(j):
            if first:
                for cp in first_group(j):
                    cp.wait()
                if j + AH < len(pairs):
                    for cp in first_group(j + AH):
                        cp.start()
                elif j + AH == len(pairs):
                    for cp in kv_copies(0, 1, 1) + [x_copy(0, 1), x_copy(1, 1)]:
                        cp.start()

        q, s, o = {}, {}, {}

        def getq(i):
            if i // 2 not in q:
                q[i // 2] = qproj(*pairs[i // 2])
            return q[i // 2]

        wait_group(-1)
        getq(0)
        getq(2)
        wait_group(0)
        s[0] = scores(getq(0), *heads[0])
        pend = []
        for i in range(n):
            if hook is not None and i == HOOK:
                hook()
            if i + 1 < n:
                if (i + 1) % 2 == 0:
                    wait_group((i + 1) // 2)
                s[i + 1] = scores(getq(i + 1), *heads[i + 1])
                if i + 3 < n:
                    getq(i + 3)
            else:
                oproj(*pend.pop(0))
            pr = softmax(s.pop(i))
            br, h = heads[i]
            o[i] = pv(pr, br, h)
            if i % 2 == 1:
                pend.append(([o.pop(i - 1), o.pop(i)], br, h // 2))
                if i + 1 == n:
                    while pend:
                        oproj(*pend.pop(0))
                elif len(pend) > 2 or (len(pend) > 1 and i + 3 < n):
                    oproj(*pend.pop(0))

    assert ahead == 1
    for j in range(-1, AH - 1):
        for cp in first_group(j):
            cp.start()

    @pl.loop(0, nb)
    def _(b):
        acc_ref[b] = jnp.zeros(acc_ref.shape[1:], acc_ref.dtype)

    body(0, 0, 0, True)

    def outer(g, slot0):
        wslot = g % 2

        @pl.when(g > 0)
        def _():
            for cp in w_copies(g, wslot):
                cp.wait()

        @pl.when(g + 1 < ng)
        def _():
            for cp in w_copies(g + 1, 1 - wslot):
                cp.start()

        def inner(b, slot):
            wrap = b + ahead >= nb
            g2 = jnp.where(wrap, g + 1, g)
            b2 = jnp.where(wrap, b + ahead - nb, b + ahead)
            slot2 = jnp.where(slot == 0, nslot - 1, slot - 1)

            def hook():
                @pl.when(g2 < ng)
                def _():
                    for cp in kv_copies(g2, b2, slot2):
                        cp.start()

                @pl.when(g2 == 0)
                def _():
                    for br in range(2):
                        x_copy(br, b2).start()

            for cp in kv_copies(g, b, slot):
                cp.wait()

            @pl.when(g == 0)
            def _():
                for br in range(2):
                    x_copy(br, b).wait()

            body(b, slot, wslot, False, hook)

            @pl.when(g == ng - 1)
            def _():
                o_buf[b] = acc_ref[b].astype(o_buf.dtype)
                o_copy(b).start()

            return jnp.where(slot == nslot - 1, 0, slot + 1)

        return jax.lax.fori_loop(jnp.where(g == 0, 1, 0), nb, inner, slot0)

    jax.lax.fori_loop(0, ng, outer, jnp.int32(1))

    for b in range(nb):
        o_copy(b).wait()


@jax.jit
def pallas_concat_heads__gqa_block_cached__gqa_block_cached__near_ridge_kernel(
    A_x, A_k_cache, A_v_cache, A_wq, A_wo, B_x, B_k_cache, B_v_cache, B_wq, B_wo):
    B, Sq, D = A_x.shape
    _, H, Sk, Dh = A_k_cache.shape
    hb = HB
    ns = NSLOT
    dt = A_x.dtype
    kt_a = jnp.swapaxes(A_k_cache, -1, -2)
    vt_a = jnp.swapaxes(A_v_cache, -1, -2)
    kt_b = jnp.swapaxes(B_k_cache, -1, -2)
    vt_b = jnp.swapaxes(B_v_cache, -1, -2)
    any_spec = pl.BlockSpec(memory_space=pl.ANY)
    dma = pltpu.SemaphoreType.DMA
    return pl.pallas_call(
        functools.partial(_kernel, hb=hb, nslot=ns),
        in_specs=[any_spec] * 10,
        out_specs=any_spec,
        out_shape=jax.ShapeDtypeStruct((B, Sq, 2 * D), dt),
        scratch_shapes=[
            pltpu.VMEM((2, B, Sq, D), dt),
            pltpu.VMEM((ns, 2, hb, Dh, Sk), dt),
            pltpu.VMEM((ns, 2, hb, Dh, Sk), dt),
            pltpu.VMEM((2, 2, D, hb * Dh), dt),
            pltpu.VMEM((2, 2, hb * Dh, D), dt),
            pltpu.VMEM((B, Sq, 2 * D), jnp.float32),
            pltpu.VMEM((B, Sq, 2 * D), dt),
            dma((2, B)), dma((ns, 2, 2)), dma((2, 2, 2)), dma((B,)),
            dma((2, 2, hb // 2)), dma((2, 2, hb // 2)),
        ],
        compiler_params=pltpu.CompilerParams(vmem_limit_bytes=110 * 1024 * 1024),
    )(A_x, B_x, kt_a, vt_a, kt_b, vt_b, A_wq, B_wq, A_wo, B_wo)
```

```python
import math

import jax
import jax.numpy as jnp
import jax.experimental.pallas as pl
import jax.experimental.pallas.tpu as pltpu

DH = 192
HB = 4

_NT = (((1,), (1,)), ((), ()))
_TN = (((0,), (0,)), ((), ()))


def _kernel(xa_hbm, xb_hbm, ka_hbm, va_hbm, kb_hbm, vb_hbm,
            wqa_hbm, wqb_hbm, woa_hbm, wob_hbm, out_hbm,
            x_buf, k_buf, v_buf, wq_buf, wo_buf, acc_ref, o_buf,
            x_sem, kv_sem, w_sem, o_sem, fkv_sem, fw_sem):
    hb = HB
    nb, _, d = xa_hbm.shape
    ng = ka_hbm.shape[1] // hb
    pw = 2 * DH
    c = (DH ** -0.5) * math.log2(math.e)
    x_hbm = (xa_hbm, xb_hbm)
    kv_hbm = ((ka_hbm, kb_hbm), (va_hbm, vb_hbm))
    kv_buf = (k_buf, v_buf)
    wq_hbm = (wqa_hbm, wqb_hbm)
    wo_hbm = (woa_hbm, wob_hbm)
    pairs = [(br, p) for p in range(hb // 2) for br in range(2)]
    heads = [(br, 2 * p + j) for br, p in pairs for j in range(2)]
    n = len(heads)

    def x_copy(br, b):
        return pltpu.make_async_copy(x_hbm[br].at[b], x_buf.at[br, b], x_sem.at[br, b])

    def kv_copies(g, b, slot):
        hs = pl.ds(g * hb, hb)
        return [pltpu.make_async_copy(kv_hbm[j][br].at[b, hs], kv_buf[j].at[slot, br],
                                      kv_sem.at[slot, br, j])
                for br in range(2) for j in range(2)]

    def w_copies(g, slot):
        cs = pl.ds(pl.multiple_of(g * (hb * DH), 128), hb * DH)
        out = []
        for br in range(2):
            out.append(pltpu.make_async_copy(wq_hbm[br].at[:, cs], wq_buf.at[slot, br],
                                             w_sem.at[slot, br, 0]))
            out.append(pltpu.make_async_copy(wo_hbm[br].at[cs, :], wo_buf.at[slot, br],
                                             w_sem.at[slot, br, 1]))
        return out

    def o_copy(b):
        return pltpu.make_async_copy(o_buf.at[b], out_hbm.at[b], o_sem.at[b])

    def fkv_copy(j, br, p):
        hs = pl.ds(2 * p, 2)
        return pltpu.make_async_copy(kv_hbm[j][br].at[0, hs], kv_buf[j].at[0, br, hs],
                                     fkv_sem.at[j, br, p])

    def fq_copy(br, p):
        cs = pl.ds(p * pw, pw)
        return pltpu.make_async_copy(wq_hbm[br].at[:, cs], wq_buf.at[0, br, :, cs],
                                     fw_sem.at[0, br, p])

    def fo_copy(br, p):
        cs = pl.ds(p * pw, pw)
        return pltpu.make_async_copy(wo_hbm[br].at[cs, :], wo_buf.at[0, br, cs, :],
                                     fw_sem.at[1, br, p])

    def first_group(j):
        if j < 0:
            return [x_copy(0, 0), fq_copy(*pairs[0]), x_copy(1, 0), fq_copy(*pairs[1])]
        out = [fkv_copy(0, *pairs[j])]
        if j + 2 < len(pairs):
            out.append(fq_copy(*pairs[j + 2]))
        return out + [fkv_copy(1, *pairs[j]), fo_copy(*pairs[j])]

    def body(b, slot, wslot, first, prefetch=None):
        def qproj(br, p):
            q = jnp.dot(x_buf[br, b], wq_buf[wslot, br, :, p * pw:(p + 1) * pw],
                        preferred_element_type=jnp.float32)
            return (q * c).astype(jnp.bfloat16)

        def scores(q, br, h):
            return jnp.dot(q[:, (h % 2) * DH:(h % 2 + 1) * DH], k_buf[slot, br, h],
                           preferred_element_type=jnp.float32)

        def softmax(s):
            m = jnp.max(s, axis=-1, keepdims=True)
            p = jnp.exp2(s - m)
            ps = p[:, 0:128]
            for j in range(1, p.shape[1] // 128):
                ps = ps + p[:, j * 128:(j + 1) * 128]
            lt = jnp.sum(jnp.transpose(ps), axis=0, keepdims=True)
            return p.astype(jnp.bfloat16), 1.0 / lt

        def pv(pr, br, h):
            p, r = pr
            ot = jax.lax.dot_general(v_buf[slot, br, h], p, _NT,
                                     preferred_element_type=jnp.float32)
            return (ot * r).astype(jnp.bfloat16)

        def oproj(j):
            br, p = pairs[j]
            ot = jnp.concatenate([o.pop(2 * j), o.pop(2 * j + 1)], axis=0)
            y = jax.lax.dot_general(ot, wo_buf[wslot, br, p * pw:(p + 1) * pw, :], _TN,
                                    preferred_element_type=jnp.float32)
            acc_ref[b, :, br * d:(br + 1) * d] += y

        def wait_group(j):
            if first:
                for cp in first_group(j):
                    cp.wait()
                if j + 2 < len(pairs):
                    for cp in first_group(j + 2):
                        cp.start()
                elif j + 2 == len(pairs):
                    for cp in kv_copies(0, 1, 1) + [x_copy(0, 1), x_copy(1, 1)]:
                        cp.start()

        q, s, o = {}, {}, {}

        def getq(i):
            if i // 2 not in q:
                q[i // 2] = qproj(*pairs[i // 2])
            return q[i // 2]

        wait_group(-1)
        getq(0)
        getq(2)
        wait_group(0)
        s[0] = scores(getq(0), *heads[0])
        for i in range(n):
            if prefetch is not None and i == 0:
                prefetch()
            if i + 1 < n:
                if (i + 1) % 2 == 0:
                    wait_group((i + 1) // 2)
                if i + 3 < n:
                    getq(i + 3)
                s[i + 1] = scores(getq(i + 1), *heads[i + 1])
            else:
                oproj(1)
            o[i] = pv(softmax(s.pop(i)), *heads[i])
            if i == 2:
                oproj(0)
        oproj(2)
        oproj(3)

    for j in (-1, 0):
        for cp in first_group(j):
            cp.start()

    @pl.loop(0, nb)
    def _(b):
        acc_ref[b] = jnp.zeros(acc_ref.shape[1:], acc_ref.dtype)

    body(0, 0, 0, True)

    def outer(g, slot0):
        wslot = g % 2

        @pl.when(g > 0)
        def _():
            for cp in w_copies(g, wslot):
                cp.wait()

        @pl.when(g + 1 < ng)
        def _():
            for cp in w_copies(g + 1, 1 - wslot):
                cp.start()

        def inner(b, slot):
            wrap = b + 1 >= nb
            g2 = jnp.where(wrap, g + 1, g)
            b2 = jnp.where(wrap, 0, b + 1)

            def prefetch():
                @pl.when(g2 < ng)
                def _():
                    for cp in kv_copies(g2, b2, 1 - slot):
                        cp.start()

                @pl.when(g2 == 0)
                def _():
                    for br in range(2):
                        x_copy(br, b2).start()

            for cp in kv_copies(g, b, slot):
                cp.wait()

            @pl.when(g == 0)
            def _():
                for br in range(2):
                    x_copy(br, b).wait()

            body(b, slot, wslot, False, prefetch)

            @pl.when(g == ng - 1)
            def _():
                o_buf[b] = acc_ref[b].astype(o_buf.dtype)
                o_copy(b).start()

            return 1 - slot

        return jax.lax.fori_loop(jnp.where(g == 0, 1, 0), nb, inner, slot0)

    jax.lax.fori_loop(0, ng, outer, jnp.int32(1))

    for b in range(nb):
        o_copy(b).wait()


@jax.jit
def pallas_concat_heads__gqa_block_cached__gqa_block_cached__near_ridge_kernel(
    A_x: jax.Array,
    A_k_cache: jax.Array,
    A_v_cache: jax.Array,
    A_wq: jax.Array,
    A_wo: jax.Array,
    B_x: jax.Array,
    B_k_cache: jax.Array,
    B_v_cache: jax.Array,
    B_wq: jax.Array,
    B_wo: jax.Array,
):
    B, Sq, D = A_x.shape
    _, H, Sk, Dh = A_k_cache.shape
    hb = HB
    assert Dh == DH and H % hb == 0 and H // hb >= 2 and B >= 2 and A_wq.shape[1] == H * Dh
    dt = A_x.dtype
    kt_a = jnp.swapaxes(A_k_cache, -1, -2)
    vt_a = jnp.swapaxes(A_v_cache, -1, -2)
    kt_b = jnp.swapaxes(B_k_cache, -1, -2)
    vt_b = jnp.swapaxes(B_v_cache, -1, -2)
    any_spec = pl.BlockSpec(memory_space=pl.ANY)
    dma = pltpu.SemaphoreType.DMA
    return pl.pallas_call(
        _kernel,
        in_specs=[any_spec] * 10,
        out_specs=any_spec,
        out_shape=jax.ShapeDtypeStruct((B, Sq, 2 * D), dt),
        scratch_shapes=[
            pltpu.VMEM((2, B, Sq, D), dt),
            pltpu.VMEM((2, 2, hb, Dh, Sk), dt),
            pltpu.VMEM((2, 2, hb, Dh, Sk), dt),
            pltpu.VMEM((2, 2, D, hb * Dh), dt),
            pltpu.VMEM((2, 2, hb * Dh, D), dt),
            pltpu.VMEM((B, Sq, 2 * D), jnp.float32),
            pltpu.VMEM((B, Sq, 2 * D), dt),
            dma((2, B)), dma((2, 2, 2)), dma((2, 2, 2)), dma((B,)),
            dma((2, 2, hb // 2)), dma((2, 2, hb // 2)),
        ],
        compiler_params=pltpu.CompilerParams(
            vmem_limit_bytes=110 * 1024 * 1024, disable_bounds_checks=True),
    )(A_x, B_x, kt_a, vt_a, kt_b, vt_b, A_wq, B_wq, A_wo, B_wo)
```
